```python
import os as _os
_os.environ.setdefault("JAX_PLATFORMS", "cpu")
import jax
import jax.numpy as jnp

def _softmax(x, axis=-1):
    return jax.nn.softmax(x, axis=axis)
def _gelu(x):
    return jax.nn.gelu(x, approximate=True)
def _silu(x):
    return jax.nn.silu(x)
def _sigmoid(x):
    return jax.nn.sigmoid(x)
def _layernorm(x, axis=-1, eps=1e-5):
    m = jnp.mean(x, axis=axis, keepdims=True)
    v = jnp.var(x, axis=axis, keepdims=True)
    return (x - m) / jnp.sqrt(v + eps)
def _scatter_add(tgt, idx, src, axis=0):
    return tgt.at[idx].add(src)
def _segment_sum(src, seg, n):
    return jax.ops.segment_sum(src, seg, n)
class _Rng:
    def __init__(self, key):
        self._k = key
    def _next(self):
        self._k, sub = jax.random.split(self._k)
        return sub
    def normal(self, shape):
        return jax.random.normal(self._next(), shape, dtype=jnp.bfloat16)
    def randint(self, lo, hi, shape):
        return jax.random.randint(self._next(), shape, lo, hi, dtype=jnp.int32)
    def uniform(self, shape, lo=0.0, hi=1.0):
        return jax.random.uniform(self._next(), shape, jnp.bfloat16, lo, hi)
    def permutation(self, n):
        return jax.random.permutation(self._next(), n)


kernel_name = 'sequential_preLN__softmax_full_mha__dense_activation_gelu__prompt'

def setup_inputs():
    _rng = _Rng(jax.random.key(int.from_bytes(__import__("os").urandom(4), "little")))
    _w = (lambda a: (lambda t: t.astype(jnp.bfloat16) if jnp.issubdtype(t.dtype, jnp.floating) else t)(jnp.asarray(a)))
    def _A_setup():
        B, S, D = 1, 2048, 640
        return {
            "x": _w((lambda *s: _rng.normal(s) * 0.05)(B, S, D)),
            "wqkv": _w((lambda *s: _rng.normal(s) * 0.05)(D, 3 * D)),
            "wo": _w((lambda *s: _rng.normal(s) * 0.05)(D, D)),
        }
    _A_in = _A_setup()

    def _B_setup():
        B, S, D, F = 1, 2048, 640, 1536
        return {
            "x": _w((lambda *s: _rng.normal(s) * 0.05)(B, S, D)),
            "w1": _w((lambda *s: _rng.normal(s) * 0.4)(D, F) * (D ** -0.5)),
            "b1": _w((lambda *s: _rng.normal(s) * 0.4)(F) * 0.01),
            "w2": _w((lambda *s: _rng.normal(s) * 0.4)(F, D) * (F ** -0.5)),
            "b2": _w((lambda *s: _rng.normal(s) * 0.05)(D) * 0.01),
        }
    _B_in = _B_setup()

    return {
        "A_x": _A_in["x"],
        "A_wqkv": _A_in["wqkv"],
        "A_wo": _A_in["wo"],
        "B_x": _B_in["x"],
        "B_w1": _B_in["w1"],
        "B_b1": _B_in["b1"],
        "B_w2": _B_in["w2"],
        "B_b2": _B_in["b2"],
    }

def reference(A_x, A_wqkv, A_wo, B_x, B_w1, B_b1, B_w2, B_b2):
    def _A_ref(x, wqkv, wo):
        B, S, D = x.shape
        H = 32; Dh = D // H
        qkv = (lambda x, *d: x.transpose(*d))((x @ wqkv).reshape(B, S, 3, H, Dh), 2, 0, 3, 1, 4)
        q, k, v = qkv[0], qkv[1], qkv[2]
        scale = Dh ** -0.5
        scores = jnp.einsum("bhqd,bhkd->bhqk", q, k) * scale
        p = _softmax(scores, axis=-1)
        o = jnp.einsum("bhqk,bhkd->bhqd", p, v)
        return (lambda x, *d: x.transpose(*d))(o, 0, 2, 1, 3).reshape(B, S, D) @ wo

    def _B_ref(x, w1, b1, w2, b2):
        h = jnp.einsum("bsd,df->bsf", x, w1) + b1
        h = _gelu(h)
        return jnp.einsum("bsf,fd->bsd", h, w2) + b2

    x = A_x
    h = x + _A_ref(_layernorm(x, axis=-1), A_wqkv, A_wo)
    h2 = h + _B_ref(_layernorm(h, axis=-1), B_w1, B_b1, B_w2, B_b2)
    return h2
```

```python
import jax
import jax.numpy as jnp
import numpy as np
import jax.experimental.pallas as pl
import jax.experimental.pallas.tpu as pltpu

S, D, F, H, DH = 2048, 640, 1536, 32, 20
NT = D // 128
NG = 2 * NT - 1
UN = 3
SUB = 128
BQ = 512
CK = 128
BR = 512
BX = 512
EPS = 1e-5
QSCALE = float(DH ** -0.5 * np.log2(np.e))
_NT = (((1,), (1,)), ((), ()))
f32, bf16 = jnp.float32, jnp.bfloat16


def _layernorm(x):
    m = jnp.mean(x, axis=-1, keepdims=True)
    xc = x - m
    v = jnp.mean(xc * xc, axis=-1, keepdims=True)
    return xc * jax.lax.rsqrt(v + EPS)


def _gelu(x):
    c = float(np.sqrt(2.0 / np.pi))
    u = x * (c + (c * 0.044715) * (x * x))
    hx = 0.5 * x
    return hx + hx * jnp.tanh(u)


def _kernel(x_hbm, wqkv_hbm, wo_hbm, w1_hbm, w2_hbm, b1_ref, b2_ref, o_ref,
            x_v, wqkv_v, wo_v, w1_v, w2_v, wqt_s, wvt_s,
            k_s, qt_s, vt_s, s_s, ot_s, sems):
    step = pl.program_id(0)

    @pl.when(step == 0)
    def _attention():
        nx = S // BX
        cp_w = pltpu.make_async_copy(wqkv_hbm, wqkv_v, sems.at[0])
        cp_x = [pltpu.make_async_copy(x_hbm.at[pl.ds(i * BX, BX)],
                                      x_v.at[pl.ds(i * BX, BX)], sems.at[4 + i])
                for i in range(nx)]
        cp_late = [pltpu.make_async_copy(wo_hbm, wo_v, sems.at[1]),
                   pltpu.make_async_copy(w1_hbm, w1_v, sems.at[2]),
                   pltpu.make_async_copy(w2_hbm, w2_v, sems.at[3])]
        cp_w.start()
        cp_x[0].start()
        cp_w.wait()
        for c in cp_x[1:]:
            c.start()
        wqt_s[...] = wqkv_v[:, :D].T
        wvt_s[...] = wqkv_v[:, 2 * D:].T

        sub = jax.lax.broadcasted_iota(jnp.int32, (8, BX), 0)
        lane = jax.lax.broadcasted_iota(jnp.int32, (SUB, 128), 1)

        def project(i, _):
            rows = pl.ds(pl.multiple_of(i * BX, BX), BX)
            pltpu.make_async_copy(x_hbm.at[rows], x_v.at[rows], sems.at[4 + i]).wait()
            xn = jnp.concatenate(
                [_layernorm(x_v[pl.ds(pl.multiple_of(i * BX + r, SUB), SUB), :]
                            .astype(f32)).astype(bf16) for r in range(0, BX, SUB)], axis=0)
            for r in range(0, BX, SUB):
                rr = pl.ds(pl.multiple_of(i * BX + r, SUB), SUB)
                k = jnp.dot(xn[r:r + SUB], wqkv_v[:, D:2 * D], preferred_element_type=f32)
                kt = [k[:, 128 * g:128 * (g + 1)] for g in range(NT)]
                for g in range(NT):
                    k_s[g, rr, :] = kt[g].astype(bf16)
                for b in range(NT - 1):
                    k_s[NT + b, rr, :] = jnp.where(lane < 64, kt[b + 1], kt[b]).astype(bf16)
            qt = jax.lax.dot_general(wqt_s[...], xn, _NT, preferred_element_type=f32)
            qt = (qt * QSCALE).astype(bf16)
            qt_s[0:D, rows] = qt
            for b in range(NT - 1):
                c = 128 * (b + 1)
                qt_s[D + 128 * b:D + 128 * b + 64, rows] = qt[c:c + 64]
                qt_s[D + 128 * b + 64:D + 128 * b + 128, rows] = qt[c - 64:c]
            vt = jax.lax.dot_general(wvt_s[...], xn, _NT, preferred_element_type=f32)
            vt = vt.astype(bf16).astype(f32)
            for p in range(H // 2):
                r = 40 * p
                mid = vt[r + 16:r + 24]
                vt_s[2 * p, 0:16, rows] = vt[r:r + 16]
                vt_s[2 * p, 16:24, rows] = jnp.where(sub < 4, mid, 1.0)
                vt_s[2 * p + 1, 0:8, rows] = jnp.where(sub < 4, 1.0, mid)
                vt_s[2 * p + 1, 8:24, rows] = vt[r + 24:r + 40]

        jax.lax.fori_loop(0, nx, project, None)
        for c in cp_late:
            c.start()

        row = jax.lax.broadcasted_iota(jnp.int32, (128, BQ), 0)
        subq = jax.lax.broadcasted_iota(jnp.int32, (8, BQ), 0)
        nsteps = H * (S // BQ)

        def load_q(t):
            h = t % H
            g = (h * DH) // 128
            lo = (h * DH) % 128
            g = jnp.where(lo + DH > 128, g + NT, g)
            cols = pl.ds(pl.multiple_of((t // H) * BQ, BQ), BQ)
            q = qt_s[pl.ds(pl.multiple_of(g * 128, 128), 128), cols]
            keep = ((row - lo) & 127) < DH
            return g, jnp.where(keep, q, jnp.zeros_like(q))

        def head_step(t, m_prev, do_qk=True, do_pv=True):
            if do_qk:
                g, q = load_q(t + 1)
            h = t % H
            m = acc = None
            for j in range(S // CK):
                keys = slice(j * CK, (j + 1) * CK)
                if do_pv:
                    p = jnp.exp2(s_s[keys, :] - m_prev).astype(bf16)
                if do_qk:
                    s = jnp.dot(k_s[g, keys, :], q, preferred_element_type=f32)
                    s_s[keys, :] = s
                    mj = jnp.max(s.reshape(CK // 8, 8, BQ), axis=0)
                    m = mj if m is None else jnp.maximum(m, mj)
                if do_pv:
                    o = jnp.dot(vt_s[h, :, keys], p, preferred_element_type=f32)
                    acc = o if acc is None else acc + o
            if do_qk:
                m = jnp.max(m, axis=0, keepdims=True)
            return acc, m

        def pair(i, m, last=False):
            t = 2 * i
            oe, m = head_step(t, m)
            oo, m = head_step(t + 1, m, do_qk=not last)
            oe = oe * (1.0 / oe[20:21])
            oo = oo * (1.0 / oo[0:1])
            o = jnp.concatenate(
                [oe[0:16], jnp.where(subq < 4, oe[16:24], oo[0:8]), oo[8:24]], axis=0)
            cols = pl.ds(pl.multiple_of((t // H) * BQ, BQ), BQ)
            ot_s[pl.ds(pl.multiple_of((i % (H // 2)) * 40, 8), 40), cols] = o
            return m

        _, m0 = head_step(-1, None, do_pv=False)
        def pairs(i, m):
            for u in range(UN):
                m = pair(i * UN + u, m)
            return m

        m0 = jax.lax.fori_loop(0, (nsteps // 2 - 1) // UN, pairs, m0)
        pair(nsteps // 2 - 1, m0, last=True)
        for c in cp_late:
            c.wait()

    b1 = b1_ref[...].astype(f32).reshape(1, F)
    b2 = b2_ref[...].astype(f32).reshape(1, D)
    hs = []
    for r in range(0, BR, SUB):
        rows = pl.ds(pl.multiple_of(step * BR + r, SUB), SUB)
        o = ot_s[:, rows].T.astype(bf16)
        hs.append(x_v[rows, :].astype(f32)
                  + jnp.dot(o, wo_v[...], preferred_element_type=f32))
    acts = []
    for h in hs:
        hn = _layernorm(h).astype(bf16)
        a = jnp.dot(hn, w1_v[...], preferred_element_type=f32) + b1
        acts.append(_gelu(a).astype(bf16))
    for n, (h, a) in enumerate(zip(hs, acts)):
        y = jnp.dot(a, w2_v[...], preferred_element_type=f32) + b2
        o_ref[n * SUB:(n + 1) * SUB, :] = (h + y).astype(o_ref.dtype)


@jax.jit
def pallas_sequential_preLN__softmax_full_mha__dense_activation_gelu__prompt_kernel(
    A_x: jax.Array,
    A_wqkv: jax.Array,
    A_wo: jax.Array,
    B_x: jax.Array,
    B_w1: jax.Array,
    B_b1: jax.Array,
    B_w2: jax.Array,
    B_b2: jax.Array,
):
    del B_x
    hbm = pl.BlockSpec(memory_space=pl.ANY)
    out = pl.pallas_call(
        _kernel,
        grid=(S // BR,),
        in_specs=[hbm, hbm, hbm, hbm, hbm,
                  pl.BlockSpec((F,), lambda i: (0,)),
                  pl.BlockSpec((D,), lambda i: (0,))],
        out_specs=pl.BlockSpec((BR, D), lambda i: (i, 0)),
        out_shape=jax.ShapeDtypeStruct((S, D), A_x.dtype),
        scratch_shapes=[
            pltpu.VMEM((S, D), bf16),
            pltpu.VMEM((D, 3 * D), bf16),
            pltpu.VMEM((D, D), bf16),
            pltpu.VMEM((D, F), bf16),
            pltpu.VMEM((F, D), bf16),
            pltpu.VMEM((D, D), bf16),
            pltpu.VMEM((D, D), bf16),
            pltpu.VMEM((NG, S, 128), bf16),
            pltpu.VMEM((NG * 128, S), bf16),
            pltpu.VMEM((H, 24, S), f32),
            pltpu.VMEM((S, BQ), f32),
            pltpu.VMEM((D, S), f32),
            pltpu.SemaphoreType.DMA((4 + S // BX,)),
        ],
        compiler_params=pltpu.CompilerParams(
            dimension_semantics=("arbitrary",),
            vmem_limit_bytes=100 * 1024 * 1024,
        ),
    )(A_x.reshape(S, D), A_wqkv, A_wo, B_w1, B_w2, B_b1, B_b2)
    return out.reshape(1, S, D)
```
